```python
import os as _os
_os.environ.setdefault("JAX_PLATFORMS", "cpu")
import jax
import jax.numpy as jnp

def _softmax(x, axis=-1):
    return jax.nn.softmax(x, axis=axis)
def _gelu(x):
    return jax.nn.gelu(x, approximate=True)
def _silu(x):
    return jax.nn.silu(x)
def _sigmoid(x):
    return jax.nn.sigmoid(x)
def _layernorm(x, axis=-1, eps=1e-5):
    m = jnp.mean(x, axis=axis, keepdims=True)
    v = jnp.var(x, axis=axis, keepdims=True)
    return (x - m) / jnp.sqrt(v + eps)
def _scatter_add(tgt, idx, src, axis=0):
    return tgt.at[idx].add(src)
def _segment_sum(src, seg, n):
    return jax.ops.segment_sum(src, seg, n)
class _Rng:
    def __init__(self, key):
        self._k = key
    def _next(self):
        self._k, sub = jax.random.split(self._k)
        return sub
    def normal(self, shape):
        return jax.random.normal(self._next(), shape, dtype=jnp.bfloat16)
    def randint(self, lo, hi, shape):
        return jax.random.randint(self._next(), shape, lo, hi, dtype=jnp.int32)
    def uniform(self, shape, lo=0.0, hi=1.0):
        return jax.random.uniform(self._next(), shape, jnp.bfloat16, lo, hi)
    def permutation(self, n):
        return jax.random.permutation(self._next(), n)


kernel_name = 'sequential_preLN__sliding_local_dilated__dense_activation_mish__prompt'

def setup_inputs():
    _rng = _Rng(jax.random.key(int.from_bytes(__import__("os").urandom(4), "little")))
    _w = (lambda a: (lambda t: t.astype(jnp.bfloat16) if jnp.issubdtype(t.dtype, jnp.floating) else t)(jnp.asarray(a)))
    def _A_setup():
        B, S, D = 1, 2048, 512
        return {
            "x": _w((lambda *s: _rng.normal(s) * 0.05)(B, S, D)),
            "wqkv": _w((lambda *s: _rng.normal(s) * 0.05)(D, 3 * D)),
            "wo": _w((lambda *s: _rng.normal(s) * 0.05)(D, D)),
        }
    _A_in = _A_setup()

    def _B_setup():
        B, S, D, F = 1, 2048, 512, 1376
        return {
            "x": _w((lambda *s: _rng.normal(s) * 0.05)(B, S, D)),
            "w1": _w((lambda *s: _rng.normal(s) * 1.6)(D, F) * (D ** -0.5)),
            "b1": _w((lambda *s: _rng.normal(s) * 0.1)(F)),
            "w2": _w((lambda *s: _rng.normal(s) * 0.1)(F, D) * (F ** -0.5)),
        }
    _B_in = _B_setup()

    return {
        "A_x": _A_in["x"],
        "A_wqkv": _A_in["wqkv"],
        "A_wo": _A_in["wo"],
        "B_x": _B_in["x"],
        "B_w1": _B_in["w1"],
        "B_b1": _B_in["b1"],
        "B_w2": _B_in["w2"],
    }

def reference(A_x, A_wqkv, A_wo, B_x, B_w1, B_b1, B_w2):
    def _A_ref(x, wqkv, wo):
        B, S, D = x.shape
        H = 32; Dh = D // H
        W, dil = 8, 2
        qkv = (lambda x, *d: x.transpose(*d))((x @ wqkv).reshape(B, S, 3, H, Dh), 2, 0, 3, 1, 4)
        q, k, v = qkv[0], qkv[1], qkv[2]
        scale = Dh ** -0.5
        pos = jnp.arange(S)
        off = jnp.arange(W) * dil
        idx = pos[:, None] - off[None, :]
        mask = idx >= 0
        idx_c = jnp.where(mask, idx, 0).reshape(-1)
        kg = k[:, :, idx_c, :].reshape(B, H, S, W, Dh)
        vg = v[:, :, idx_c, :].reshape(B, H, S, W, Dh)
        logits = jnp.einsum("bhsd,bhswd->bhsw", q, kg) * scale
        logits = jnp.where(mask[None, None, :, :], logits, -1e9)
        attn = _softmax(logits, axis=-1)
        o = jnp.einsum("bhsw,bhswd->bhsd", attn, vg)
        return (lambda x, *d: x.transpose(*d))(o, 0, 2, 1, 3).reshape(B, S, D) @ wo

    def _B_ref(x, w1, b1, w2):
        h = jnp.einsum("bsd,df->bsf", x, w1) + b1
        sp = jnp.log1p(jnp.exp(-jnp.abs(h))) + jnp.where(h > 0, h, jnp.zeros_like(h))
        act = h * jnp.tanh(sp)
        return jnp.einsum("bsf,fd->bsd", act, w2)

    x = A_x
    h = x + _A_ref(_layernorm(x, axis=-1), A_wqkv, A_wo)
    h2 = h + _B_ref(_layernorm(h, axis=-1), B_w1, B_b1, B_w2)
    return h2
```

```python
import jax
import jax.numpy as jnp
import numpy as np
from jax import lax
import jax.experimental.pallas as pl
import jax.experimental.pallas.tpu as pltpu

S, D, H, DH, F = 2048, 512, 32, 16, 1376
NW, DIL = 8, 2
HALO = 16
EPS = 1e-5
LOG2E = 1.4426950408889634
QSCALE = (DH ** -0.5) * LOG2E
QBITS = int(np.float32(QSCALE).view(np.int32))
NEG = -1e9 * LOG2E
f32, bf16, i32 = jnp.float32, jnp.bfloat16, jnp.int32

T = 256
NT = S // T
RA = 16
RL = 64
RC = 64
FCH = 128
F2M = 128
CHAIN = 4
N_F1 = len(range(0, F, FCH))


def _ln(x):
    m = jnp.sum(x, axis=-1, keepdims=True) * (1.0 / D)
    d = x - m
    v = jnp.sum(d * d, axis=-1, keepdims=True) * (1.0 / D)
    return d * lax.rsqrt(v + EPS)


def _mish(h):
    n = jnp.exp2(jnp.minimum(h, 20.0) * LOG2E)
    u = n * (n + 2.0)
    return h * u * pltpu.reciprocal(u + 2.0, approx=True)


def _ld16(ref, r0, nr, c0=None, c1=None):
    if c0 is None:
        return pltpu.bitcast(ref[r0 // 2:(r0 + nr) // 2, :], bf16)
    return pltpu.bitcast(ref[r0 // 2:(r0 + nr) // 2, c0:c1], bf16)


def _st16(ref, r0, nr, c0, c1, val):
    ref[r0 // 2:(r0 + nr) // 2, c0:c1] = pltpu.bitcast(val.astype(bf16), i32)


class _Gen:
    def __init__(self, g, n):
        self.g, self.n, self.i = g, n, 0


def _interleave(*gens):
    start = [s.i for s in gens]
    while True:
        live = [k for k, s in enumerate(gens) if s.i < s.n]
        if not live:
            return
        k = min(live, key=lambda k: (gens[k].i - start[k] + 0.5) / (gens[k].n - start[k]))
        next(gens[k].g)
        gens[k].i += 1


def _kernel(x_hbm, wqkv_hbm, wo_hbm, w1t_hbm, b1_hbm, w2_hbm, out_hbm,
            x_ref, wqkv_ref, wo_ref, w1t_ref, b1_ref, w2_ref, out_ref,
            wp_ref, wop_ref, w1p_ref, w2p_ref, bf_ref, tmp_ref, q_ref, k_ref, v_ref,
            xn_ref, o_ref, h_ref, hn_ref, act_ref,
            sem_x, sem_w, sem_o, sem_l):

    def rows_copy(src, dst, r0, n, sem):
        return pltpu.make_async_copy(src.at[pl.ds(r0, n), :], dst.at[pl.ds(r0, n), :], sem)

    def wqkv_copy(p):
        return pltpu.make_async_copy(wqkv_hbm.at[:, pl.ds(p * D, D)],
                                     wqkv_ref.at[:, pl.ds(p * D, D)], sem_w.at[p])

    wo_copy = pltpu.make_async_copy(wo_hbm, wo_ref, sem_w.at[3])
    w1_copy = pltpu.make_async_copy(w1t_hbm, w1t_ref, sem_w.at[4])
    b1_copy = pltpu.make_async_copy(b1_hbm, b1_ref, sem_w.at[5])
    w2_copy = pltpu.make_async_copy(w2_hbm, w2_ref, sem_w.at[6])
    xs = [rows_copy(x_hbm, x_ref, i * T, T, sem_x.at[i]) for i in range(4)]
    xr = rows_copy(x_hbm, x_ref, 4 * T, S - 4 * T, sem_x.at[4])

    def out_copy(t):
        return rows_copy(out_ref, out_hbm, t * T, T, sem_o.at[t])

    def permute_part(p):
        def g_():
            lane = lax.broadcasted_iota(i32, (RC // 2, 128), 1)
            quad = (lane % 16) // 4
            g = lane // 32
            b = (lane % 32) // 8
            hl = lane % 8
            for c in range(4):
                idx = hl * 16 + 4 * ((b + c) % 4) + g
                for r in range(0, D, RC):
                    blks = [pltpu.bitcast(wqkv_ref[r:r + RC, p * D + bb * 128:p * D + (bb + 1) * 128], i32)
                            for bb in range(4)]
                    xx = blks[(0 - c) % 4]
                    for qd in range(1, 4):
                        xx = jnp.where(quad == qd, blks[(qd - c) % 4], xx)
                    wp_ref[r // 2:(r + RC) // 2, p * D + c * 128:p * D + (c + 1) * 128] = (
                        jnp.take_along_axis(xx, idx, axis=1))
                yield
        return _Gen(g_(), 4)

    wo_gate = []

    def permute_wo():
        def g_():
            for j in range(4):
                for r in range(0, D, 64):
                    tmp_ref[j, r:r + 64, :] = wo_ref[r:r + 64, j * 128:(j + 1) * 128].astype(f32)
                yield
            for j in range(4):
                for c in range(4):
                    for g in range(4):
                        parts = [tmp_ref[j, pl.ds(128 * b + 4 * ((b + c) % 4) + g, 8, stride=16), :]
                                 for b in range(4)]
                        v = jnp.concatenate(parts, axis=0)
                        _st16(wop_ref, c * 128 + 32 * g, 32, j * 128, (j + 1) * 128, v)
                        if j == 3 and c == 3 and g == 3:
                            wo_gate.append(jnp.abs(v[0:RA, :]))
                yield
        return _Gen(g_(), 8)

    def repack(src_ref, dst_ref):
        def g_():
            for r in range(0, F, RC):
                n = min(RC, F - r)
                dst_ref[r // 2:(r + n) // 2, :] = pltpu.bitcast(src_ref[r:r + n, :], i32)
                yield
        return _Gen(g_(), len(range(0, F, RC)))

    def ln1(t):
        def g_():
            for r in range(t * T, (t + 1) * T, RL):
                _st16(xn_ref, r, RL, 0, D, _ln(x_ref[r:r + RL, :].astype(f32)))
                yield
        return _Gen(g_(), T // RL)

    def qkv(t, parts=(0, 1, 2)):
        def g_():
            r0 = t * T
            for p in parts:
                for c in range(4):
                    y = jnp.dot(_ld16(xn_ref, r0, T),
                                _ld16(wp_ref, 0, D, p * D + c * 128, p * D + (c + 1) * 128),
                                preferred_element_type=f32)
                    if p == 0:
                        q_ref[c, r0:r0 + T, :] = y
                    elif p == 1:
                        k_ref[c, HALO + r0:HALO + r0 + T, :] = y
                    else:
                        v_ref[c, HALO + r0:HALO + r0 + T, :] = y
                    yield
        return _Gen(g_(), 4 * len(parts))

    def halo():
        for c in range(4):
            k_ref[c, 0:HALO, :] = jnp.broadcast_to(k_ref[c, HALO:HALO + 1, :], (HALO, 128))
            v_ref[c, 0:HALO, :] = jnp.broadcast_to(v_ref[c, HALO:HALO + 1, :], (HALO, 128))

    links = []

    def attn(t):
        def g_():
            for r0 in range(t * T, (t + 1) * T, RA):
                u = (r0 - t * T) // RA
                q = [q_ref[c, r0:r0 + RA, :] for c in range(4)]
                prev = None
                if t == 0 and u < CHAIN:
                    prev = wo_gate[0]
                elif len(links) >= CHAIN:
                    prev = links[-CHAIN]
                if prev is not None:
                    cvec = pltpu.bitcast(
                        lax.shift_right_logical(pltpu.bitcast(prev, i32), 31) | QBITS, f32)
                    q = [qq * cvec for qq in q]
                else:
                    q = [qq * QSCALE for qq in q]
                logits = []
                for w in range(NW):
                    s = None
                    for c in range(4):
                        kk = k_ref[c, pl.ds(HALO + r0 - DIL * w, RA), :]
                        s = q[c] * kk if s is None else s + q[c] * kk
                    s = s + pltpu.roll(s, 64, 1)
                    s = s + pltpu.roll(s, 32, 1)
                    if w > 0 and r0 < DIL * w:
                        rows = lax.broadcasted_iota(i32, (RA, 128), 0) + r0
                        s = jnp.where(rows >= DIL * w, s, NEG)
                    logits.append(s)
                m = logits[0]
                for w in range(1, NW):
                    m = jnp.maximum(m, logits[w])
                e = [jnp.exp2(l - m) for l in logits]
                den = e[0]
                for w in range(1, NW):
                    den = den + e[w]
                rcp = pltpu.reciprocal(den, approx=True)
                links.append(rcp)
                for c in range(4):
                    acc = None
                    for w in range(NW):
                        vv = v_ref[c, pl.ds(HALO + r0 - DIL * w, RA), :]
                        acc = e[w] * vv if acc is None else acc + e[w] * vv
                    _st16(o_ref, r0, RA, c * 128, (c + 1) * 128, acc * rcp)
                yield
        return _Gen(g_(), T // RA)

    def wo(t):
        def g_():
            r0 = t * T
            for c in range(4):
                y = jnp.dot(_ld16(o_ref, r0, T), _ld16(wop_ref, 0, D, c * 128, (c + 1) * 128),
                            preferred_element_type=f32)
                h_ref[r0:r0 + T, c * 128:(c + 1) * 128] = (
                    x_ref[r0:r0 + T, c * 128:(c + 1) * 128].astype(f32) + y)
                yield
        return _Gen(g_(), 4)

    def ln2(t):
        def g_():
            for r in range(t * T, (t + 1) * T, RL):
                _st16(hn_ref, r, RL, 0, D, _ln(h_ref[r:r + RL, :]))
                yield
        return _Gen(g_(), T // RL)

    def ffn1(t):
        def g_():
            r0 = t * T
            for f0 in range(0, F, FCH):
                f1 = min(F, f0 + FCH)
                y = lax.dot_general(_ld16(hn_ref, r0, T), _ld16(w1p_ref, f0, f1 - f0),
                                    (((1,), (1,)), ((), ())), preferred_element_type=f32)
                _st16(act_ref, r0, T, f0, f1, _mish(y + bf_ref[:, f0:f1]))
                yield
        return _Gen(g_(), N_F1)

    def ffn2(t):
        def g_():
            for n0 in range(0, D, 128):
                for r0 in range(t * T, (t + 1) * T, F2M):
                    y = jnp.dot(_ld16(act_ref, r0, F2M), _ld16(w2p_ref, 0, F, n0, n0 + 128),
                                preferred_element_type=f32)
                    out_ref[r0:r0 + F2M, n0:n0 + 128] = (h_ref[r0:r0 + F2M, n0:n0 + 128] + y).astype(bf16)
                yield
        return _Gen(g_(), 4)

    xs[0].start()
    wqkv_copy(0).start()
    xs[0].wait()
    xs[1].start()
    _interleave(ln1(0))
    wqkv_copy(0).wait()
    wqkv_copy(1).start()
    q0 = qkv(0, (0,))
    q0.n = 2
    _interleave(permute_part(0), q0)
    xs[1].wait()
    wqkv_copy(2).start()
    q0.n = 4
    _interleave(q0, ln1(1))
    q1 = qkv(1, (0,))
    q1.n = 2
    _interleave(q1)
    wqkv_copy(1).wait()
    xs[2].start()
    wo_copy.start()
    q1.n = 4
    _interleave(permute_part(1), q1)
    _interleave(qkv(0, (1,)))
    k1 = qkv(1, (1,))
    k1.n = 2
    _interleave(k1)
    wqkv_copy(2).wait()
    w1_copy.start()
    b1_copy.start()
    k1.n = 4
    _interleave(permute_part(2), k1)
    _interleave(qkv(0, (2,)))
    halo()
    v1 = qkv(1, (2,))
    v1.n = 2
    _interleave(v1)
    xs[2].wait()
    wo_copy.wait()
    xs[3].start()
    w2_copy.start()
    v1.n = 4
    _interleave(v1, ln1(2), permute_wo())

    f2 = None
    for t in range(NT):
        gens = [attn(t)]
        if t == 0:
            gens.append(qkv(2, (0, 1)))
        elif t + 2 < NT:
            gens.append(qkv(t + 2))
        else:
            f2 = ffn2(t - 1)
            f2.n = 2
            gens.append(f2)
        _interleave(*gens)
        _interleave(wo(t))
        gens = [ln2(t)]
        if t == 0:
            w1_copy.wait()
            b1_copy.wait()
            xs[3].wait()
            xr.start()
            bf_ref[...] = b1_ref[...].astype(f32).reshape(1, F)
            gens += [qkv(2, (2,)), repack(w1t_ref, w1p_ref)]
        elif t == 1:
            _interleave(repack(w2_ref, w2p_ref))
            gens.append(ffn2(t - 1))
        elif t + 2 >= NT:
            f2.n = 4
            gens.append(f2)
        else:
            gens.append(ffn2(t - 1))
        if t + 3 < NT:
            gens.append(ln1(t + 3))
        _interleave(*gens)
        if t >= 1:
            out_copy(t - 1).start()
        _interleave(ffn1(t))
        if t == 0:
            w2_copy.wait()
            xr.wait()

    tl = NT - 1
    last = []
    g = ffn2(tl)
    for c in range(4):
        next(g.g)
        cp = pltpu.make_async_copy(out_ref.at[pl.ds(tl * T, T), pl.ds(c * 128, 128)],
                                   out_hbm.at[pl.ds(tl * T, T), pl.ds(c * 128, 128)], sem_l.at[c])
        cp.start()
        last.append(cp)
    for t in range(NT - 1):
        out_copy(t).wait()
    for cp in last:
        cp.wait()


@jax.jit
def pallas_sequential_preLN__sliding_local_dilated__dense_activation_mish__prompt_kernel(
    A_x: jax.Array,
    A_wqkv: jax.Array,
    A_wo: jax.Array,
    B_x: jax.Array,
    B_w1: jax.Array,
    B_b1: jax.Array,
    B_w2: jax.Array,
):
    del B_x
    hbm = pl.BlockSpec(memory_space=pltpu.HBM)
    out = pl.pallas_call(
        _kernel,
        in_specs=[hbm] * 6,
        out_specs=hbm,
        out_shape=jax.ShapeDtypeStruct((S, D), bf16),
        scratch_shapes=[
            pltpu.VMEM((S, D), bf16),
            pltpu.VMEM((D, 3 * D), bf16),
            pltpu.VMEM((D, D), bf16),
            pltpu.VMEM((F, D), bf16),
            pltpu.VMEM((F,), bf16),
            pltpu.VMEM((F, D), bf16),
            pltpu.VMEM((S, D), bf16),
            pltpu.VMEM((D // 2, 3 * D), i32),
            pltpu.VMEM((D // 2, D), i32),
            pltpu.VMEM((F // 2, D), i32),
            pltpu.VMEM((F // 2, D), i32),
            pltpu.VMEM((1, F), f32),
            pltpu.VMEM((4, D, 128), f32),
            pltpu.VMEM((4, S, 128), f32),
            pltpu.VMEM((4, HALO + S, 128), f32),
            pltpu.VMEM((4, HALO + S, 128), f32),
            pltpu.VMEM((S // 2, D), i32),
            pltpu.VMEM((S // 2, D), i32),
            pltpu.VMEM((S, D), f32),
            pltpu.VMEM((S // 2, D), i32),
            pltpu.VMEM((S // 2, F), i32),
            pltpu.SemaphoreType.DMA((5,)),
            pltpu.SemaphoreType.DMA((7,)),
            pltpu.SemaphoreType.DMA((NT,)),
            pltpu.SemaphoreType.DMA((4,)),
        ],
        compiler_params=pltpu.CompilerParams(vmem_limit_bytes=100 * 1024 * 1024),
    )(A_x.reshape(S, D), A_wqkv, A_wo, B_w1.T, B_b1, B_w2)
    return out.reshape(1, S, D)
```

```python
import jax
import jax.numpy as jnp
import numpy as np
from jax import lax
import jax.experimental.pallas as pl
import jax.experimental.pallas.tpu as pltpu

S, D, H, DH, F = 2048, 512, 32, 16, 1376
NW, DIL = 8, 2
HALO = 16
EPS = 1e-5
LOG2E = 1.4426950408889634
QSCALE = (DH ** -0.5) * LOG2E
QBITS = int(np.float32(QSCALE).view(np.int32))
NEG = -1e9 * LOG2E
f32, bf16, i32 = jnp.float32, jnp.bfloat16, jnp.int32

T = 256
NT = S // T
RA = 16
RL = 64
RC = 64
FCH = 128
F2M = 128
CHAIN = (4, 5, 6, 6, 6, 6, 5, 5)
N_F1 = len(range(0, F, FCH))


def _ln(x):
    m = jnp.sum(x, axis=-1, keepdims=True) * (1.0 / D)
    d = x - m
    v = jnp.sum(d * d, axis=-1, keepdims=True) * (1.0 / D)
    return d * lax.rsqrt(v + EPS)


def _mish(h):
    n = jnp.exp2(jnp.minimum(h, 20.0) * LOG2E)
    u = n * (n + 2.0)
    return h * u * pltpu.reciprocal(u + 2.0, approx=True)


def _ld16(ref, r0, nr, c0=None, c1=None):
    if c0 is None:
        return pltpu.bitcast(ref[r0 // 2:(r0 + nr) // 2, :], bf16)
    return pltpu.bitcast(ref[r0 // 2:(r0 + nr) // 2, c0:c1], bf16)


def _st16(ref, r0, nr, c0, c1, val):
    ref[r0 // 2:(r0 + nr) // 2, c0:c1] = pltpu.bitcast(val.astype(bf16), i32)


class _Gen:
    def __init__(self, g, n):
        self.g, self.n, self.i = g, n, 0


def _interleave(*gens):
    start = [s.i for s in gens]
    while True:
        live = [k for k, s in enumerate(gens) if s.i < s.n]
        if not live:
            return
        k = min(live, key=lambda k: (gens[k].i - start[k] + 0.5) / (gens[k].n - start[k]))
        next(gens[k].g)
        gens[k].i += 1


def _kernel(x_hbm, wqkv_hbm, wo_hbm, w1t_hbm, b1_hbm, w2_hbm, out_hbm,
            x_ref, wqkv_ref, wo_ref, w1t_ref, b1_ref, w2_ref, out_ref,
            wp_ref, wop_ref, w1p_ref, w2p_ref, bf_ref, tmp_ref, q_ref, k_ref, v_ref,
            xn_ref, o_ref, h_ref, hn_ref, act_ref,
            sems):

    def rows_copy(src, dst, r0, n, sem):
        return pltpu.make_async_copy(src.at[pl.ds(r0, n), :], dst.at[pl.ds(r0, n), :], sem)

    sem_a, sem_b, sem_o = sems.at[0], sems.at[1], sems.at[2]

    def wqkv_copy(p):
        return pltpu.make_async_copy(wqkv_hbm.at[:, pl.ds(p * D, D)],
                                     wqkv_ref.at[:, pl.ds(p * D, D)], (sem_b, sem_b, sem_a)[p])

    wo_copy = pltpu.make_async_copy(wo_hbm, wo_ref, sem_b)
    w1_copy = pltpu.make_async_copy(w1t_hbm, w1t_ref, sem_a)
    b1_copy = pltpu.make_async_copy(b1_hbm, b1_ref, sem_a)
    w2_copy = pltpu.make_async_copy(w2_hbm, w2_ref, sem_b)
    xs = [rows_copy(x_hbm, x_ref, i * T, T, (sem_a, sem_a, sem_b, sem_a)[i]) for i in range(4)]
    xr = rows_copy(x_hbm, x_ref, 4 * T, S - 4 * T, sem_a)

    def out_copy(t):
        return rows_copy(out_ref, out_hbm, t * T, T, sem_o)

    def permute_part(p):
        def g_():
            lane = lax.broadcasted_iota(i32, (RC // 2, 128), 1)
            quad = (lane % 16) // 4
            g = lane // 32
            b = (lane % 32) // 8
            hl = lane % 8
            for c in range(4):
                idx = hl * 16 + 4 * ((b + c) % 4) + g
                for r in range(0, D, RC):
                    blks = [pltpu.bitcast(wqkv_ref[r:r + RC, p * D + bb * 128:p * D + (bb + 1) * 128], i32)
                            for bb in range(4)]
                    xx = blks[(0 - c) % 4]
                    for qd in range(1, 4):
                        xx = jnp.where(quad == qd, blks[(qd - c) % 4], xx)
                    wp_ref[r // 2:(r + RC) // 2, p * D + c * 128:p * D + (c + 1) * 128] = (
                        jnp.take_along_axis(xx, idx, axis=1))
                yield
        return _Gen(g_(), 4)

    wo_gate = []

    def permute_wo():
        def g_():
            for j in range(4):
                for r in range(0, D, 64):
                    tmp_ref[j, r:r + 64, :] = wo_ref[r:r + 64, j * 128:(j + 1) * 128].astype(f32)
                yield
            for j in range(4):
                for c in range(4):
                    for g in range(4):
                        parts = [tmp_ref[j, pl.ds(128 * b + 4 * ((b + c) % 4) + g, 8, stride=16), :]
                                 for b in range(4)]
                        v = jnp.concatenate(parts, axis=0)
                        _st16(wop_ref, c * 128 + 32 * g, 32, j * 128, (j + 1) * 128, v)
                        if j == 3 and c == 3 and g == 3:
                            wo_gate.append(jnp.abs(v[0:RA, :]))
                yield
        return _Gen(g_(), 8)

    def repack(src_ref, dst_ref):
        def g_():
            for r in range(0, F, RC):
                n = min(RC, F - r)
                dst_ref[r // 2:(r + n) // 2, :] = pltpu.bitcast(src_ref[r:r + n, :], i32)
                yield
        return _Gen(g_(), len(range(0, F, RC)))

    def ln1(t):
        def g_():
            for r in range(t * T, (t + 1) * T, RL):
                _st16(xn_ref, r, RL, 0, D, _ln(x_ref[r:r + RL, :].astype(f32)))
                yield
        return _Gen(g_(), T // RL)

    def qkv(t, parts=(0, 1, 2)):
        def g_():
            r0 = t * T
            for p in parts:
                for c in range(4):
                    y = jnp.dot(_ld16(xn_ref, r0, T),
                                _ld16(wp_ref, 0, D, p * D + c * 128, p * D + (c + 1) * 128),
                                preferred_element_type=f32)
                    if p == 0:
                        q_ref[c, r0:r0 + T, :] = y
                    elif p == 1:
                        k_ref[c, HALO + r0:HALO + r0 + T, :] = y
                    else:
                        v_ref[c, HALO + r0:HALO + r0 + T, :] = y
                    yield
        return _Gen(g_(), 4 * len(parts))

    def halo():
        for c in range(4):
            k_ref[c, 0:HALO, :] = jnp.broadcast_to(k_ref[c, HALO:HALO + 1, :], (HALO, 128))
            v_ref[c, 0:HALO, :] = jnp.broadcast_to(v_ref[c, HALO:HALO + 1, :], (HALO, 128))

    links = []

    def attn(t):
        def g_():
            for r0 in range(t * T, (t + 1) * T, RA):
                u = (r0 - t * T) // RA
                q = [q_ref[c, r0:r0 + RA, :] for c in range(4)]
                prev = None
                if t == 0 and u < CHAIN[t]:
                    prev = wo_gate[0]
                elif len(links) >= CHAIN[t]:
                    prev = links[-CHAIN[t]]
                if prev is not None:
                    cvec = pltpu.bitcast(
                        lax.shift_right_logical(pltpu.bitcast(prev, i32), 31) | QBITS, f32)
                    q = [qq * cvec for qq in q]
                else:
                    q = [qq * QSCALE for qq in q]
                logits = []
                for w in range(NW):
                    s = None
                    for c in range(4):
                        kk = k_ref[c, pl.ds(HALO + r0 - DIL * w, RA), :]
                        s = q[c] * kk if s is None else s + q[c] * kk
                    s = s + pltpu.roll(s, 64, 1)
                    s = s + pltpu.roll(s, 32, 1)
                    if w > 0 and r0 < DIL * w:
                        rows = lax.broadcasted_iota(i32, (RA, 128), 0) + r0
                        s = jnp.where(rows >= DIL * w, s, NEG)
                    logits.append(s)
                m = logits[0]
                for w in range(1, NW):
                    m = jnp.maximum(m, logits[w])
                e = [jnp.exp2(l - m) for l in logits]
                den = e[0]
                for w in range(1, NW):
                    den = den + e[w]
                rcp = pltpu.reciprocal(den, approx=True)
                links.append(rcp)
                for c in range(4):
                    acc = None
                    for w in range(NW):
                        vv = v_ref[c, pl.ds(HALO + r0 - DIL * w, RA), :]
                        acc = e[w] * vv if acc is None else acc + e[w] * vv
                    _st16(o_ref, r0, RA, c * 128, (c + 1) * 128, acc * rcp)
                yield
        return _Gen(g_(), T // RA)

    def wo(t):
        def g_():
            r0 = t * T
            for c in range(4):
                y = jnp.dot(_ld16(o_ref, r0, T), _ld16(wop_ref, 0, D, c * 128, (c + 1) * 128),
                            preferred_element_type=f32)
                h_ref[r0:r0 + T, c * 128:(c + 1) * 128] = (
                    x_ref[r0:r0 + T, c * 128:(c + 1) * 128].astype(f32) + y)
                yield
        return _Gen(g_(), 4)

    def ln2(t):
        def g_():
            for r in range(t * T, (t + 1) * T, RL):
                _st16(hn_ref, r, RL, 0, D, _ln(h_ref[r:r + RL, :]))
                yield
        return _Gen(g_(), T // RL)

    def ffn1(t):
        def g_():
            r0 = t * T
            for f0 in range(0, F, FCH):
                f1 = min(F, f0 + FCH)
                y = lax.dot_general(_ld16(hn_ref, r0, T), _ld16(w1p_ref, f0, f1 - f0),
                                    (((1,), (1,)), ((), ())), preferred_element_type=f32)
                _st16(act_ref, r0, T, f0, f1, _mish(y + bf_ref[:, f0:f1]))
                yield
        return _Gen(g_(), N_F1)

    def ffn2(t):
        def g_():
            for n0 in range(0, D, 128):
                for r0 in range(t * T, (t + 1) * T, F2M):
                    y = jnp.dot(_ld16(act_ref, r0, F2M), _ld16(w2p_ref, 0, F, n0, n0 + 128),
                                preferred_element_type=f32)
                    out_ref[r0:r0 + F2M, n0:n0 + 128] = (h_ref[r0:r0 + F2M, n0:n0 + 128] + y).astype(bf16)
                yield
        return _Gen(g_(), 4)

    xs[0].start()
    wqkv_copy(0).start()
    xs[0].wait()
    xs[1].start()
    _interleave(ln1(0))
    wqkv_copy(0).wait()
    wqkv_copy(1).start()
    q0 = qkv(0, (0,))
    q0.n = 2
    _interleave(permute_part(0), q0)
    xs[1].wait()
    wqkv_copy(2).start()
    q0.n = 4
    _interleave(q0, ln1(1))
    q1 = qkv(1, (0,))
    q1.n = 3
    _interleave(q1)
    wqkv_copy(1).wait()
    xs[2].start()
    wo_copy.start()
    q1.n = 4
    _interleave(permute_part(1), q1)
    _interleave(qkv(0, (1,)))
    k1 = qkv(1, (1,))
    k1.n = 2
    _interleave(k1)
    wqkv_copy(2).wait()
    w1_copy.start()
    b1_copy.start()
    k1.n = 4
    _interleave(permute_part(2), k1)
    _interleave(qkv(0, (2,)))
    halo()
    v1 = qkv(1, (2,))
    v1.n = 1
    _interleave(v1)
    xs[2].wait()
    wo_copy.wait()
    xs[3].start()
    w2_copy.start()
    v1.n = 4
    _interleave(v1, ln1(2), permute_wo())

    f2 = None
    for t in range(NT):
        gens = [attn(t)]
        if t == 0:
            gens.append(qkv(2, (0, 1)))
        elif t + 2 < NT:
            gens.append(qkv(t + 2))
        else:
            f2 = ffn2(t - 1)
            f2.n = 2
            gens.append(f2)
        _interleave(*gens)
        _interleave(wo(t))
        gens = [ln2(t)]
        if t == 0:
            w1_copy.wait()
            b1_copy.wait()
            xs[3].wait()
            xr.start()
            bf_ref[...] = b1_ref[...].astype(f32).reshape(1, F)
            gens += [qkv(2, (2,)), repack(w1t_ref, w1p_ref)]
        elif t == 1:
            _interleave(repack(w2_ref, w2p_ref))
            gens.append(ffn2(t - 1))
        elif t + 2 >= NT:
            f2.n = 4
            gens.append(f2)
        else:
            gens.append(ffn2(t - 1))
        if t + 3 < NT:
            gens.append(ln1(t + 3))
        _interleave(*gens)
        if t >= 1:
            out_copy(t - 1).start()
        _interleave(ffn1(t))
        if t == 0:
            w2_copy.wait()
            xr.wait()

    tl = NT - 1
    g = ffn2(tl)
    for c in range(4):
        next(g.g)
        pltpu.make_async_copy(out_ref.at[pl.ds(tl * T, T), pl.ds(c * 128, 128)],
                              out_hbm.at[pl.ds(tl * T, T), pl.ds(c * 128, 128)], sem_o).start()
    pltpu.make_async_copy(out_ref, out_hbm, sem_o).wait()


@jax.jit
def pallas_sequential_preLN__sliding_local_dilated__dense_activation_mish__prompt_kernel(
    A_x: jax.Array,
    A_wqkv: jax.Array,
    A_wo: jax.Array,
    B_x: jax.Array,
    B_w1: jax.Array,
    B_b1: jax.Array,
    B_w2: jax.Array,
):
    del B_x
    hbm = pl.BlockSpec(memory_space=pltpu.HBM)
    out = pl.pallas_call(
        _kernel,
        in_specs=[hbm] * 6,
        out_specs=hbm,
        out_shape=jax.ShapeDtypeStruct((S, D), bf16),
        scratch_shapes=[
            pltpu.VMEM((S, D), bf16),
            pltpu.VMEM((D, 3 * D), bf16),
            pltpu.VMEM((D, D), bf16),
            pltpu.VMEM((F, D), bf16),
            pltpu.VMEM((F,), bf16),
            pltpu.VMEM((F, D), bf16),
            pltpu.VMEM((S, D), bf16),
            pltpu.VMEM((D // 2, 3 * D), i32),
            pltpu.VMEM((D // 2, D), i32),
            pltpu.VMEM((F // 2, D), i32),
            pltpu.VMEM((F // 2, D), i32),
            pltpu.VMEM((1, F), f32),
            pltpu.VMEM((4, D, 128), f32),
            pltpu.VMEM((4, S, 128), f32),
            pltpu.VMEM((4, HALO + S, 128), f32),
            pltpu.VMEM((4, HALO + S, 128), f32),
            pltpu.VMEM((S // 2, D), i32),
            pltpu.VMEM((S // 2, D), i32),
            pltpu.VMEM((S, D), f32),
            pltpu.VMEM((S // 2, D), i32),
            pltpu.VMEM((S // 2, F), i32),
            pltpu.SemaphoreType.DMA((3,)),
        ],
        compiler_params=pltpu.CompilerParams(vmem_limit_bytes=100 * 1024 * 1024),
    )(A_x.reshape(S, D), A_wqkv, A_wo, B_w1.T, B_b1, B_w2)
    return out.reshape(1, S, D)
```

```python
import jax
import jax.numpy as jnp
import numpy as np
from jax import lax
import jax.experimental.pallas as pl
import jax.experimental.pallas.tpu as pltpu

S, D, H, DH, F = 2048, 512, 32, 16, 1376
NW, DIL = 8, 2
HALO = 16
EPS = 1e-5
LOG2E = 1.4426950408889634
QSCALE = (DH ** -0.5) * LOG2E
QBITS = int(np.float32(QSCALE).view(np.int32))
NEG = -1e9 * LOG2E
f32, bf16, i32 = jnp.float32, jnp.bfloat16, jnp.int32

T = 256
NT = S // T
RA = 16
RL = 64
RC = 64
FCH = 128
F2M = 128
CHAIN = (4, 5, 6, 6, 6, 6, 5, 5)
N_F1 = len(range(0, F, FCH))


def _ln(x):
    m = jnp.sum(x, axis=-1, keepdims=True) * (1.0 / D)
    d = x - m
    v = jnp.sum(d * d, axis=-1, keepdims=True) * (1.0 / D)
    return d * lax.rsqrt(v + EPS)


def _mish(h):
    n = jnp.exp2(jnp.minimum(h, 20.0) * LOG2E)
    u = n * (n + 2.0)
    return h * u * pltpu.reciprocal(u + 2.0, approx=True)


def _ld16(ref, r0, nr, c0=None, c1=None):
    if c0 is None:
        return pltpu.bitcast(ref[r0 // 2:(r0 + nr) // 2, :], bf16)
    return pltpu.bitcast(ref[r0 // 2:(r0 + nr) // 2, c0:c1], bf16)


def _st16(ref, r0, nr, c0, c1, val):
    ref[r0 // 2:(r0 + nr) // 2, c0:c1] = pltpu.bitcast(val.astype(bf16), i32)


class _Gen:
    def __init__(self, g, n):
        self.g, self.n, self.i = g, n, 0


def _interleave(*gens):
    start = [s.i for s in gens]
    while True:
        live = [k for k, s in enumerate(gens) if s.i < s.n]
        if not live:
            return
        k = min(live, key=lambda k: (gens[k].i - start[k] + 0.5) / (gens[k].n - start[k]))
        next(gens[k].g)
        gens[k].i += 1


def _kernel(x_hbm, wqkv_hbm, wo_hbm, w1t_hbm, b1_hbm, w2_hbm, out_hbm,
            x_ref, wqkv_ref, wo_ref, w1t_ref, b1_ref, w2_ref, out_ref,
            wp_ref, wop_ref, w1p_ref, w2p_ref, bf_ref, tmp_ref, q_ref, k_ref, v_ref,
            xn_ref, o_ref, h_ref, hn_ref, act_ref,
            sems):

    def rows_copy(src, dst, r0, n, sem):
        return pltpu.make_async_copy(src.at[pl.ds(r0, n), :], dst.at[pl.ds(r0, n), :], sem)

    sem_a, sem_b, sem_o = sems.at[0], sems.at[1], sems.at[2]

    def wqkv_copy(p):
        return pltpu.make_async_copy(wqkv_hbm.at[:, pl.ds(p * D, D)],
                                     wqkv_ref.at[:, pl.ds(p * D, D)], (sem_b, sem_b, sem_a)[p])

    wo_copy = pltpu.make_async_copy(wo_hbm, wo_ref, sem_b)
    w1_copy = pltpu.make_async_copy(w1t_hbm, w1t_ref, sem_a)
    b1_copy = pltpu.make_async_copy(b1_hbm, b1_ref, sem_a)
    w2_copy = pltpu.make_async_copy(w2_hbm, w2_ref, sem_b)
    xs = [rows_copy(x_hbm, x_ref, i * T, T, (sem_a, sem_a, sem_b, sem_a)[i]) for i in range(4)]
    xr = rows_copy(x_hbm, x_ref, 4 * T, S - 4 * T, sem_a)

    def out_copy(t):
        return rows_copy(out_ref, out_hbm, t * T, T, sem_o)

    def permute_part(p):
        def g_():
            lane = lax.broadcasted_iota(i32, (RC // 2, 128), 1)
            quad = (lane % 16) // 4
            g = lane // 32
            b = (lane % 32) // 8
            hl = lane % 8
            for c in range(4):
                idx = hl * 16 + 4 * ((b + c) % 4) + g
                for r in range(0, D, RC):
                    blks = [pltpu.bitcast(wqkv_ref[r:r + RC, p * D + bb * 128:p * D + (bb + 1) * 128], i32)
                            for bb in range(4)]
                    xx = blks[(0 - c) % 4]
                    for qd in range(1, 4):
                        xx = jnp.where(quad == qd, blks[(qd - c) % 4], xx)
                    wp_ref[r // 2:(r + RC) // 2, p * D + c * 128:p * D + (c + 1) * 128] = (
                        jnp.take_along_axis(xx, idx, axis=1))
                yield
        return _Gen(g_(), 4)

    wo_gate = []

    def permute_wo():
        def g_():
            for j in range(4):
                for r in range(0, D, 64):
                    tmp_ref[j, r:r + 64, :] = wo_ref[r:r + 64, j * 128:(j + 1) * 128].astype(f32)
                yield
            for j in range(4):
                for c in range(4):
                    for g in range(4):
                        parts = [tmp_ref[j, pl.ds(128 * b + 4 * ((b + c) % 4) + g, 8, stride=16), :]
                                 for b in range(4)]
                        v = jnp.concatenate(parts, axis=0)
                        _st16(wop_ref, c * 128 + 32 * g, 32, j * 128, (j + 1) * 128, v)
                        if j == 3 and c == 3 and g == 3:
                            wo_gate.append(jnp.abs(v[0:RA, :]))
                yield
        return _Gen(g_(), 8)

    def repack(src_ref, dst_ref):
        def g_():
            for r in range(0, F, RC):
                n = min(RC, F - r)
                dst_ref[r // 2:(r + n) // 2, :] = pltpu.bitcast(src_ref[r:r + n, :], i32)
                yield
        return _Gen(g_(), len(range(0, F, RC)))

    def ln1(t):
        def g_():
            for r in range(t * T, (t + 1) * T, RL):
                _st16(xn_ref, r, RL, 0, D, _ln(x_ref[r:r + RL, :].astype(f32)))
                yield
        return _Gen(g_(), T // RL)

    def qkv(t, parts=(0, 1, 2)):
        def g_():
            r0 = t * T
            for p in parts:
                for c in range(4):
                    y = jnp.dot(_ld16(xn_ref, r0, T),
                                _ld16(wp_ref, 0, D, p * D + c * 128, p * D + (c + 1) * 128),
                                preferred_element_type=f32)
                    if p == 0:
                        q_ref[c, r0:r0 + T, :] = y
                    elif p == 1:
                        k_ref[c, HALO + r0:HALO + r0 + T, :] = y
                    else:
                        v_ref[c, HALO + r0:HALO + r0 + T, :] = y
                    yield
        return _Gen(g_(), 4 * len(parts))

    def halo():
        for c in range(4):
            k_ref[c, 0:HALO, :] = jnp.broadcast_to(k_ref[c, HALO:HALO + 1, :], (HALO, 128))
            v_ref[c, 0:HALO, :] = jnp.broadcast_to(v_ref[c, HALO:HALO + 1, :], (HALO, 128))

    links = []

    def attn(t):
        def g_():
            for r0 in range(t * T, (t + 1) * T, RA):
                u = (r0 - t * T) // RA
                q = [q_ref[c, r0:r0 + RA, :] for c in range(4)]
                prev = None
                if t == 0 and u < CHAIN[t]:
                    prev = wo_gate[0]
                elif len(links) >= CHAIN[t]:
                    prev = links[-CHAIN[t]]
                if prev is not None:
                    cvec = pltpu.bitcast(
                        lax.shift_right_logical(pltpu.bitcast(prev, i32), 31) | QBITS, f32)
                    q = [qq * cvec for qq in q]
                else:
                    q = [qq * QSCALE for qq in q]
                logits = []
                for w in range(NW):
                    s = None
                    for c in range(4):
                        kk = k_ref[c, pl.ds(HALO + r0 - DIL * w, RA), :]
                        s = q[c] * kk if s is None else s + q[c] * kk
                    s = s + pltpu.roll(s, 64, 1)
                    s = s + pltpu.roll(s, 32, 1)
                    if w > 0 and r0 < DIL * w:
                        rows = lax.broadcasted_iota(i32, (RA, 128), 0) + r0
                        s = jnp.where(rows >= DIL * w, s, NEG)
                    logits.append(s)
                m = logits[0]
                for w in range(1, NW):
                    m = jnp.maximum(m, logits[w])
                e = [jnp.exp2(l - m) for l in logits]
                den = e[0]
                for w in range(1, NW):
                    den = den + e[w]
                rcp = pltpu.reciprocal(den, approx=True)
                links.append(rcp)
                for c in range(4):
                    acc = None
                    for w in range(NW):
                        vv = v_ref[c, pl.ds(HALO + r0 - DIL * w, RA), :]
                        acc = e[w] * vv if acc is None else acc + e[w] * vv
                    _st16(o_ref, r0, RA, c * 128, (c + 1) * 128, acc * rcp)
                yield
        return _Gen(g_(), T // RA)

    def wo(t):
        def g_():
            r0 = t * T
            for c in range(4):
                y = jnp.dot(_ld16(o_ref, r0, T), _ld16(wop_ref, 0, D, c * 128, (c + 1) * 128),
                            preferred_element_type=f32)
                h_ref[r0:r0 + T, c * 128:(c + 1) * 128] = (
                    x_ref[r0:r0 + T, c * 128:(c + 1) * 128].astype(f32) + y)
                yield
        return _Gen(g_(), 4)

    def ln2(t):
        def g_():
            for r in range(t * T, (t + 1) * T, RL):
                _st16(hn_ref, r, RL, 0, D, _ln(h_ref[r:r + RL, :]))
                yield
        return _Gen(g_(), T // RL)

    def ffn1(t):
        def g_():
            r0 = t * T
            for f0 in range(0, F, FCH):
                f1 = min(F, f0 + FCH)
                y = lax.dot_general(_ld16(hn_ref, r0, T), _ld16(w1p_ref, f0, f1 - f0),
                                    (((1,), (1,)), ((), ())), preferred_element_type=f32)
                _st16(act_ref, r0, T, f0, f1, _mish(y + bf_ref[:, f0:f1]))
                yield
        return _Gen(g_(), N_F1)

    def ffn2(t):
        def g_():
            for n0 in range(0, D, 128):
                for r0 in range(t * T, (t + 1) * T, F2M):
                    y = jnp.dot(_ld16(act_ref, r0, F2M), _ld16(w2p_ref, 0, F, n0, n0 + 128),
                                preferred_element_type=f32)
                    out_ref[r0:r0 + F2M, n0:n0 + 128] = (h_ref[r0:r0 + F2M, n0:n0 + 128] + y).astype(bf16)
                yield
        return _Gen(g_(), 4)

    xs[0].start()
    wqkv_copy(0).start()
    xs[0].wait()
    xs[1].start()
    _interleave(ln1(0))
    wqkv_copy(0).wait()
    wqkv_copy(1).start()
    q0 = qkv(0, (0,))
    q0.n = 2
    _interleave(permute_part(0), q0)
    xs[1].wait()
    wqkv_copy(2).start()
    q0.n = 4
    _interleave(q0, ln1(1))
    q1 = qkv(1, (0,))
    q1.n = 3
    _interleave(q1)
    wqkv_copy(1).wait()
    xs[2].start()
    wo_copy.start()
    q1.n = 4
    _interleave(permute_part(1), q1)
    _interleave(qkv(0, (1,)))
    k1 = qkv(1, (1,))
    k1.n = 2
    _interleave(k1)
    wqkv_copy(2).wait()
    w1_copy.start()
    b1_copy.start()
    k1.n = 4
    _interleave(permute_part(2), k1)
    _interleave(qkv(0, (2,)))
    halo()
    v1 = qkv(1, (2,))
    v1.n = 1
    _interleave(v1)
    xs[2].wait()
    wo_copy.wait()
    xs[3].start()
    w2_copy.start()
    v1.n = 4
    _interleave(v1, ln1(2), permute_wo())

    for t in range(NT):
        gens = [attn(t)]
        if t == 0:
            gens.append(qkv(2, (0, 1)))
        elif t + 2 < NT:
            gens.append(qkv(t + 2))
        _interleave(*gens)
        _interleave(wo(t))
        gens = [ln2(t)]
        if t == 0:
            w1_copy.wait()
            b1_copy.wait()
            xs[3].wait()
            xr.start()
            bf_ref[...] = b1_ref[...].astype(f32).reshape(1, F)
            gens += [qkv(2, (2,)), repack(w1t_ref, w1p_ref)]
        else:
            if t == 1:
                _interleave(repack(w2_ref, w2p_ref))
            gens.append(ffn2(t - 1))
        if t + 3 < NT:
            gens.append(ln1(t + 3))
        _interleave(*gens)
        if t >= 1:
            out_copy(t - 1).start()
        _interleave(ffn1(t))
        if t == 0:
            w2_copy.wait()
            xr.wait()

    tl = NT - 1
    g = ffn2(tl)
    for c in range(4):
        next(g.g)
        pltpu.make_async_copy(out_ref.at[pl.ds(tl * T, T), pl.ds(c * 128, 128)],
                              out_hbm.at[pl.ds(tl * T, T), pl.ds(c * 128, 128)], sem_o).start()
    pltpu.make_async_copy(out_ref, out_hbm, sem_o).wait()


@jax.jit
def pallas_sequential_preLN__sliding_local_dilated__dense_activation_mish__prompt_kernel(
    A_x: jax.Array,
    A_wqkv: jax.Array,
    A_wo: jax.Array,
    B_x: jax.Array,
    B_w1: jax.Array,
    B_b1: jax.Array,
    B_w2: jax.Array,
):
    del B_x
    hbm = pl.BlockSpec(memory_space=pltpu.HBM)
    out = pl.pallas_call(
        _kernel,
        in_specs=[hbm] * 6,
        out_specs=hbm,
        out_shape=jax.ShapeDtypeStruct((S, D), bf16),
        scratch_shapes=[
            pltpu.VMEM((S, D), bf16),
            pltpu.VMEM((D, 3 * D), bf16),
            pltpu.VMEM((D, D), bf16),
            pltpu.VMEM((F, D), bf16),
            pltpu.VMEM((F,), bf16),
            pltpu.VMEM((F, D), bf16),
            pltpu.VMEM((S, D), bf16),
            pltpu.VMEM((D // 2, 3 * D), i32),
            pltpu.VMEM((D // 2, D), i32),
            pltpu.VMEM((F // 2, D), i32),
            pltpu.VMEM((F // 2, D), i32),
            pltpu.VMEM((1, F), f32),
            pltpu.VMEM((4, D, 128), f32),
            pltpu.VMEM((4, S, 128), f32),
            pltpu.VMEM((4, HALO + S, 128), f32),
            pltpu.VMEM((4, HALO + S, 128), f32),
            pltpu.VMEM((S // 2, D), i32),
            pltpu.VMEM((S // 2, D), i32),
            pltpu.VMEM((S, D), f32),
            pltpu.VMEM((S // 2, D), i32),
            pltpu.VMEM((S // 2, F), i32),
            pltpu.SemaphoreType.DMA((3,)),
        ],
        compiler_params=pltpu.CompilerParams(vmem_limit_bytes=100 * 1024 * 1024),
    )(A_x.reshape(S, D), A_wqkv, A_wo, B_w1.T, B_b1, B_w2)
    return out.reshape(1, S, D)
```

```python
import jax
import jax.numpy as jnp
import numpy as np
from jax import lax
import jax.experimental.pallas as pl
import jax.experimental.pallas.tpu as pltpu

S, D, H, DH, F = 2048, 512, 32, 16, 1376
NW, DIL = 8, 2
HALO = 16
EPS = 1e-5
LOG2E = 1.4426950408889634
QSCALE = (DH ** -0.5) * LOG2E
QBITS = int(np.float32(QSCALE).view(np.int32))
NEG = -1e9 * LOG2E
f32, bf16, i32 = jnp.float32, jnp.bfloat16, jnp.int32

T = 256
NT = S // T
RA = 16
RL = 64
RC = 64
FCH = 128
F2M = 128
TAILM = 64
CHAIN = (4, 5, 6, 6, 6, 6, 5, 5)
N_F1 = len(range(0, F, FCH))


def _ln(x):
    m = jnp.sum(x, axis=-1, keepdims=True) * (1.0 / D)
    d = x - m
    v = jnp.sum(d * d, axis=-1, keepdims=True) * (1.0 / D)
    return d * lax.rsqrt(v + EPS)


def _mish(h):
    n = jnp.exp2(jnp.minimum(h, 20.0) * LOG2E)
    u = n * (n + 2.0)
    return h * u * pltpu.reciprocal(u + 2.0, approx=True)


def _ld16(ref, r0, nr, c0=None, c1=None):
    if c0 is None:
        return pltpu.bitcast(ref[r0 // 2:(r0 + nr) // 2, :], bf16)
    return pltpu.bitcast(ref[r0 // 2:(r0 + nr) // 2, c0:c1], bf16)


def _st16(ref, r0, nr, c0, c1, val):
    ref[r0 // 2:(r0 + nr) // 2, c0:c1] = pltpu.bitcast(val.astype(bf16), i32)


class _Gen:
    def __init__(self, g, n):
        self.g, self.n, self.i = g, n, 0


def _interleave(*gens):
    start = [s.i for s in gens]
    while True:
        live = [k for k, s in enumerate(gens) if s.i < s.n]
        if not live:
            return
        k = min(live, key=lambda k: (gens[k].i - start[k] + 0.5) / (gens[k].n - start[k]))
        next(gens[k].g)
        gens[k].i += 1


def _kernel(x_hbm, wqkv_hbm, wo_hbm, w1t_hbm, b1_hbm, w2_hbm, out_hbm,
            x_ref, wqkv_ref, wo_ref, w1t_ref, b1_ref, w2_ref, out_ref,
            wp_ref, wop_ref, w1p_ref, w2p_ref, bf_ref, tmp_ref, q_ref, k_ref, v_ref,
            xn_ref, o_ref, h_ref, hn_ref, act_ref,
            sems):

    def rows_copy(src, dst, r0, n, sem):
        return pltpu.make_async_copy(src.at[pl.ds(r0, n), :], dst.at[pl.ds(r0, n), :], sem)

    sem_a, sem_b, sem_o = sems.at[0], sems.at[1], sems.at[2]

    def wqkv_copy(p):
        return pltpu.make_async_copy(wqkv_hbm.at[:, pl.ds(p * D, D)],
                                     wqkv_ref.at[:, pl.ds(p * D, D)], (sem_b, sem_b, sem_a)[p])

    wo_copy = pltpu.make_async_copy(wo_hbm, wo_ref, sem_b)
    w1_copy = pltpu.make_async_copy(w1t_hbm, w1t_ref, sem_a)
    b1_copy = pltpu.make_async_copy(b1_hbm, b1_ref, sem_a)
    w2_copy = pltpu.make_async_copy(w2_hbm, w2_ref, sem_b)
    xs = [rows_copy(x_hbm, x_ref, i * T, T, (sem_a, sem_a, sem_b, sem_a)[i]) for i in range(4)]
    xr = rows_copy(x_hbm, x_ref, 4 * T, S - 4 * T, sem_a)

    def out_copy(t):
        return rows_copy(out_ref, out_hbm, t * T, T, sem_o)

    def permute_part(p):
        def g_():
            lane = lax.broadcasted_iota(i32, (RC // 2, 128), 1)
            quad = (lane % 16) // 4
            g = lane // 32
            b = (lane % 32) // 8
            hl = lane % 8
            for c in range(4):
                idx = hl * 16 + 4 * ((b + c) % 4) + g
                for r in range(0, D, RC):
                    blks = [pltpu.bitcast(wqkv_ref[r:r + RC, p * D + bb * 128:p * D + (bb + 1) * 128], i32)
                            for bb in range(4)]
                    xx = blks[(0 - c) % 4]
                    for qd in range(1, 4):
                        xx = jnp.where(quad == qd, blks[(qd - c) % 4], xx)
                    wp_ref[r // 2:(r + RC) // 2, p * D + c * 128:p * D + (c + 1) * 128] = (
                        jnp.take_along_axis(xx, idx, axis=1))
                yield
        return _Gen(g_(), 4)

    wo_gate = []

    def permute_wo():
        def g_():
            for j in range(4):
                for r in range(0, D, 64):
                    tmp_ref[j, r:r + 64, :] = wo_ref[r:r + 64, j * 128:(j + 1) * 128].astype(f32)
                yield
            for j in range(4):
                for c in range(4):
                    for g in range(4):
                        parts = [tmp_ref[j, pl.ds(128 * b + 4 * ((b + c) % 4) + g, 8, stride=16), :]
                                 for b in range(4)]
                        v = jnp.concatenate(parts, axis=0)
                        _st16(wop_ref, c * 128 + 32 * g, 32, j * 128, (j + 1) * 128, v)
                        if j == 3 and c == 3 and g == 3:
                            wo_gate.append(jnp.abs(v[0:RA, :]))
                yield
        return _Gen(g_(), 8)

    def repack(src_ref, dst_ref):
        def g_():
            for r in range(0, F, RC):
                n = min(RC, F - r)
                dst_ref[r // 2:(r + n) // 2, :] = pltpu.bitcast(src_ref[r:r + n, :], i32)
                yield
        return _Gen(g_(), len(range(0, F, RC)))

    def ln1(t):
        def g_():
            for r in range(t * T, (t + 1) * T, RL):
                _st16(xn_ref, r, RL, 0, D, _ln(x_ref[r:r + RL, :].astype(f32)))
                yield
        return _Gen(g_(), T // RL)

    def qkv(t, parts=(0, 1, 2)):
        def g_():
            r0 = t * T
            for p in parts:
                for c in range(4):
                    y = jnp.dot(_ld16(xn_ref, r0, T),
                                _ld16(wp_ref, 0, D, p * D + c * 128, p * D + (c + 1) * 128),
                                preferred_element_type=f32)
                    if p == 0:
                        q_ref[c, r0:r0 + T, :] = y
                    elif p == 1:
                        k_ref[c, HALO + r0:HALO + r0 + T, :] = y
                    else:
                        v_ref[c, HALO + r0:HALO + r0 + T, :] = y
                    yield
        return _Gen(g_(), 4 * len(parts))

    def halo():
        for c in range(4):
            k_ref[c, 0:HALO, :] = jnp.broadcast_to(k_ref[c, HALO:HALO + 1, :], (HALO, 128))
            v_ref[c, 0:HALO, :] = jnp.broadcast_to(v_ref[c, HALO:HALO + 1, :], (HALO, 128))

    links = []

    def attn(t):
        def g_():
            for r0 in range(t * T, (t + 1) * T, RA):
                u = (r0 - t * T) // RA
                q = [q_ref[c, r0:r0 + RA, :] for c in range(4)]
                prev = None
                if t == 0 and u < CHAIN[t]:
                    prev = wo_gate[0]
                elif len(links) >= CHAIN[t]:
                    prev = links[-CHAIN[t]]
                if prev is not None:
                    cvec = pltpu.bitcast(
                        lax.shift_right_logical(pltpu.bitcast(prev, i32), 31) | QBITS, f32)
                    q = [qq * cvec for qq in q]
                else:
                    q = [qq * QSCALE for qq in q]
                logits = []
                for w in range(NW):
                    s = None
                    for c in range(4):
                        kk = k_ref[c, pl.ds(HALO + r0 - DIL * w, RA), :]
                        s = q[c] * kk if s is None else s + q[c] * kk
                    s = s + pltpu.roll(s, 64, 1)
                    s = s + pltpu.roll(s, 32, 1)
                    if w > 0 and r0 < DIL * w:
                        rows = lax.broadcasted_iota(i32, (RA, 128), 0) + r0
                        s = jnp.where(rows >= DIL * w, s, NEG)
                    logits.append(s)
                m = logits[0]
                for w in range(1, NW):
                    m = jnp.maximum(m, logits[w])
                e = [jnp.exp2(l - m) for l in logits]
                den = e[0]
                for w in range(1, NW):
                    den = den + e[w]
                rcp = pltpu.reciprocal(den, approx=True)
                links.append(rcp)
                for c in range(4):
                    acc = None
                    for w in range(NW):
                        vv = v_ref[c, pl.ds(HALO + r0 - DIL * w, RA), :]
                        acc = e[w] * vv if acc is None else acc + e[w] * vv
                    _st16(o_ref, r0, RA, c * 128, (c + 1) * 128, acc * rcp)
                yield
        return _Gen(g_(), T // RA)

    def wo(t):
        def g_():
            r0 = t * T
            for c in range(4):
                y = jnp.dot(_ld16(o_ref, r0, T), _ld16(wop_ref, 0, D, c * 128, (c + 1) * 128),
                            preferred_element_type=f32)
                h_ref[r0:r0 + T, c * 128:(c + 1) * 128] = (
                    x_ref[r0:r0 + T, c * 128:(c + 1) * 128].astype(f32) + y)
                yield
        return _Gen(g_(), 4)

    def ln2(t):
        def g_():
            for r in range(t * T, (t + 1) * T, RL):
                _st16(hn_ref, r, RL, 0, D, _ln(h_ref[r:r + RL, :]))
                yield
        return _Gen(g_(), T // RL)

    def ffn1(t):
        def g_():
            r0 = t * T
            for f0 in range(0, F, FCH):
                f1 = min(F, f0 + FCH)
                y = lax.dot_general(_ld16(hn_ref, r0, T), _ld16(w1p_ref, f0, f1 - f0),
                                    (((1,), (1,)), ((), ())), preferred_element_type=f32)
                _st16(act_ref, r0, T, f0, f1, _mish(y + bf_ref[:, f0:f1]))
                yield
        return _Gen(g_(), N_F1)

    def ffn2_piece(r0, nr, n0):
        y = jnp.dot(_ld16(act_ref, r0, nr), _ld16(w2p_ref, 0, F, n0, n0 + 128), preferred_element_type=f32)
        out_ref[r0:r0 + nr, n0:n0 + 128] = (h_ref[r0:r0 + nr, n0:n0 + 128] + y).astype(bf16)

    def ffn2(t):
        def g_():
            for n0 in range(0, D, 128):
                for r0 in range(t * T, (t + 1) * T, F2M):
                    ffn2_piece(r0, F2M, n0)
                yield
        return _Gen(g_(), 4)

    xs[0].start()
    wqkv_copy(0).start()
    xs[0].wait()
    xs[1].start()
    _interleave(ln1(0))
    wqkv_copy(0).wait()
    wqkv_copy(1).start()
    q0 = qkv(0, (0,))
    q0.n = 2
    _interleave(permute_part(0), q0)
    xs[1].wait()
    wqkv_copy(2).start()
    q0.n = 4
    _interleave(q0, ln1(1))
    q1 = qkv(1, (0,))
    q1.n = 3
    _interleave(q1)
    wqkv_copy(1).wait()
    xs[2].start()
    wo_copy.start()
    q1.n = 4
    _interleave(permute_part(1), q1)
    _interleave(qkv(0, (1,)))
    k1 = qkv(1, (1,))
    k1.n = 2
    _interleave(k1)
    wqkv_copy(2).wait()
    w1_copy.start()
    b1_copy.start()
    k1.n = 4
    _interleave(permute_part(2), k1)
    _interleave(qkv(0, (2,)))
    halo()
    v1 = qkv(1, (2,))
    v1.n = 1
    _interleave(v1)
    xs[2].wait()
    wo_copy.wait()
    xs[3].start()
    w2_copy.start()
    v1.n = 4
    _interleave(v1, ln1(2), permute_wo())

    for t in range(NT):
        gens = [attn(t)]
        if t == 0:
            gens.append(qkv(2, (0, 1)))
        elif t + 2 < NT:
            gens.append(qkv(t + 2))
        _interleave(*gens)
        _interleave(wo(t))
        gens = [ln2(t)]
        if t == 0:
            w1_copy.wait()
            b1_copy.wait()
            xs[3].wait()
            xr.start()
            bf_ref[...] = b1_ref[...].astype(f32).reshape(1, F)
            gens += [qkv(2, (2,)), repack(w1t_ref, w1p_ref)]
        else:
            if t == 1:
                _interleave(repack(w2_ref, w2p_ref))
            gens.append(ffn2(t - 1))
        if t + 3 < NT:
            gens.append(ln1(t + 3))
        _interleave(*gens)
        if t >= 1:
            out_copy(t - 1).start()
        _interleave(ffn1(t))
        if t == 0:
            w2_copy.wait()
            xr.wait()

    r_last = (NT - 1) * T
    for n0 in range(0, D, 128):
        for r0 in range(r_last, S, TAILM):
            ffn2_piece(r0, TAILM, n0)
            if n0 == D - 128 or r0 + TAILM == S:
                r1, nr = (r0, TAILM) if n0 == D - 128 else (r_last, T)
                pltpu.make_async_copy(out_ref.at[pl.ds(r1, nr), pl.ds(n0, 128)],
                                      out_hbm.at[pl.ds(r1, nr), pl.ds(n0, 128)], sem_o).start()
    pltpu.make_async_copy(out_ref, out_hbm, sem_o).wait()


@jax.jit
def pallas_sequential_preLN__sliding_local_dilated__dense_activation_mish__prompt_kernel(
    A_x: jax.Array,
    A_wqkv: jax.Array,
    A_wo: jax.Array,
    B_x: jax.Array,
    B_w1: jax.Array,
    B_b1: jax.Array,
    B_w2: jax.Array,
):
    del B_x
    hbm = pl.BlockSpec(memory_space=pltpu.HBM)
    out = pl.pallas_call(
        _kernel,
        in_specs=[hbm] * 6,
        out_specs=hbm,
        out_shape=jax.ShapeDtypeStruct((S, D), bf16),
        scratch_shapes=[
            pltpu.VMEM((S, D), bf16),
            pltpu.VMEM((D, 3 * D), bf16),
            pltpu.VMEM((D, D), bf16),
            pltpu.VMEM((F, D), bf16),
            pltpu.VMEM((F,), bf16),
            pltpu.VMEM((F, D), bf16),
            pltpu.VMEM((S, D), bf16),
            pltpu.VMEM((D // 2, 3 * D), i32),
            pltpu.VMEM((D // 2, D), i32),
            pltpu.VMEM((F // 2, D), i32),
            pltpu.VMEM((F // 2, D), i32),
            pltpu.VMEM((1, F), f32),
            pltpu.VMEM((4, D, 128), f32),
            pltpu.VMEM((4, S, 128), f32),
            pltpu.VMEM((4, HALO + S, 128), f32),
            pltpu.VMEM((4, HALO + S, 128), f32),
            pltpu.VMEM((S // 2, D), i32),
            pltpu.VMEM((S // 2, D), i32),
            pltpu.VMEM((S, D), f32),
            pltpu.VMEM((S // 2, D), i32),
            pltpu.VMEM((S // 2, F), i32),
            pltpu.SemaphoreType.DMA((3,)),
        ],
        compiler_params=pltpu.CompilerParams(vmem_limit_bytes=100 * 1024 * 1024),
    )(A_x.reshape(S, D), A_wqkv, A_wo, B_w1.T, B_b1, B_w2)
    return out.reshape(1, S, D)
```

```python
import jax
import jax.numpy as jnp
import numpy as np
from jax import lax
import jax.experimental.pallas as pl
import jax.experimental.pallas.tpu as pltpu

S, D, H, DH, F = 2048, 512, 32, 16, 1376
NW, DIL = 8, 2
HALO = 16
EPS = 1e-5
LOG2E = 1.4426950408889634
QSCALE = (DH ** -0.5) * LOG2E
QBITS = int(np.float32(QSCALE).view(np.int32))
NEG = -1e9 * LOG2E
f32, bf16, i32 = jnp.float32, jnp.bfloat16, jnp.int32

T = 256
NT = S // T
RA = 16
RL = 64
RC = 64
FCH = 128
F2M = 128
TAILM = 64
CHAIN = (4, 5, 5, 5, 5, 5, 5, 5)
N_F1 = len(range(0, F, FCH))


def _ln(x):
    m = jnp.sum(x, axis=-1, keepdims=True) * (1.0 / D)
    d = x - m
    v = jnp.sum(d * d, axis=-1, keepdims=True) * (1.0 / D)
    return d * lax.rsqrt(v + EPS)


def _mish(h):
    n = jnp.exp2(jnp.minimum(h, 20.0) * LOG2E)
    u = n * (n + 2.0)
    return h * u * pltpu.reciprocal(u + 2.0, approx=True)


def _ld16(ref, r0, nr, c0=None, c1=None):
    if c0 is None:
        return pltpu.bitcast(ref[r0 // 2:(r0 + nr) // 2, :], bf16)
    return pltpu.bitcast(ref[r0 // 2:(r0 + nr) // 2, c0:c1], bf16)


def _st16(ref, r0, nr, c0, c1, val):
    ref[r0 // 2:(r0 + nr) // 2, c0:c1] = pltpu.bitcast(val.astype(bf16), i32)


class _Gen:
    def __init__(self, g, n):
        self.g, self.n, self.i = g, n, 0


def _interleave(*gens):
    start = [s.i for s in gens]
    while True:
        live = [k for k, s in enumerate(gens) if s.i < s.n]
        if not live:
            return
        k = min(live, key=lambda k: (gens[k].i - start[k] + 0.5) / (gens[k].n - start[k]))
        next(gens[k].g)
        gens[k].i += 1


def _kernel(x_hbm, wqkv_hbm, wo_hbm, w1t_hbm, b1_hbm, w2_hbm, out_hbm,
            x_ref, wqkv_ref, wo_ref, w1t_ref, b1_ref, w2_ref, out_ref,
            wp_ref, wop_ref, w1p_ref, w2p_ref, bf_ref, tmp_ref, q_ref, k_ref, v_ref,
            xn_ref, o_ref, h_ref, hn_ref, act_ref,
            sems):

    def rows_copy(src, dst, r0, n, sem):
        return pltpu.make_async_copy(src.at[pl.ds(r0, n), :], dst.at[pl.ds(r0, n), :], sem)

    sem_a, sem_b, sem_o = sems.at[0], sems.at[1], sems.at[2]

    def wqkv_copy(p):
        return pltpu.make_async_copy(wqkv_hbm.at[:, pl.ds(p * D, D)],
                                     wqkv_ref.at[:, pl.ds(p * D, D)], (sem_b, sem_b, sem_a)[p])

    wo_copy = pltpu.make_async_copy(wo_hbm, wo_ref, sem_b)
    w1_copy = pltpu.make_async_copy(w1t_hbm, w1t_ref, sem_a)
    b1_copy = pltpu.make_async_copy(b1_hbm, b1_ref, sem_a)
    w2_copy = pltpu.make_async_copy(w2_hbm, w2_ref, sem_b)
    xs = [rows_copy(x_hbm, x_ref, i * T, T, (sem_a, sem_a, sem_b, sem_a)[i]) for i in range(4)]
    xr = rows_copy(x_hbm, x_ref, 4 * T, S - 4 * T, sem_a)

    def out_copy(t):
        return rows_copy(out_ref, out_hbm, t * T, T, sem_o)

    def permute_part(p):
        def g_():
            lane = lax.broadcasted_iota(i32, (RC // 2, 128), 1)
            quad = (lane % 16) // 4
            g = lane // 32
            b = (lane % 32) // 8
            hl = lane % 8
            for c in range(4):
                idx = hl * 16 + 4 * ((b + c) % 4) + g
                for r in range(0, D, RC):
                    blks = [pltpu.bitcast(wqkv_ref[r:r + RC, p * D + bb * 128:p * D + (bb + 1) * 128], i32)
                            for bb in range(4)]
                    xx = blks[(0 - c) % 4]
                    for qd in range(1, 4):
                        xx = jnp.where(quad == qd, blks[(qd - c) % 4], xx)
                    wp_ref[r // 2:(r + RC) // 2, p * D + c * 128:p * D + (c + 1) * 128] = (
                        jnp.take_along_axis(xx, idx, axis=1))
                yield
        return _Gen(g_(), 4)

    wo_gate = []

    def permute_wo():
        def g_():
            for j in range(4):
                for r in range(0, D, 64):
                    tmp_ref[j, r:r + 64, :] = wo_ref[r:r + 64, j * 128:(j + 1) * 128].astype(f32)
                yield
            for j in range(4):
                for c in range(4):
                    for g in range(4):
                        parts = [tmp_ref[j, pl.ds(128 * b + 4 * ((b + c) % 4) + g, 8, stride=16), :]
                                 for b in range(4)]
                        v = jnp.concatenate(parts, axis=0)
                        _st16(wop_ref, c * 128 + 32 * g, 32, j * 128, (j + 1) * 128, v)
                        if j == 3 and c == 3 and g == 3:
                            wo_gate.append(jnp.abs(v[0:RA, :]))
                yield
        return _Gen(g_(), 8)

    def repack(src_ref, dst_ref):
        def g_():
            for r in range(0, F, RC):
                n = min(RC, F - r)
                dst_ref[r // 2:(r + n) // 2, :] = pltpu.bitcast(src_ref[r:r + n, :], i32)
                yield
        return _Gen(g_(), len(range(0, F, RC)))

    def ln1(t):
        def g_():
            for r in range(t * T, (t + 1) * T, RL):
                _st16(xn_ref, r, RL, 0, D, _ln(x_ref[r:r + RL, :].astype(f32)))
                yield
        return _Gen(g_(), T // RL)

    def qkv(t, parts=(0, 1, 2)):
        def g_():
            r0 = t * T
            for p in parts:
                for c in range(4):
                    y = jnp.dot(_ld16(xn_ref, r0, T),
                                _ld16(wp_ref, 0, D, p * D + c * 128, p * D + (c + 1) * 128),
                                preferred_element_type=f32)
                    if p == 0:
                        q_ref[c, r0:r0 + T, :] = y
                    elif p == 1:
                        k_ref[c, HALO + r0:HALO + r0 + T, :] = y
                    else:
                        v_ref[c, HALO + r0:HALO + r0 + T, :] = y
                    yield
        return _Gen(g_(), 4 * len(parts))

    def halo():
        for c in range(4):
            k_ref[c, 0:HALO, :] = jnp.broadcast_to(k_ref[c, HALO:HALO + 1, :], (HALO, 128))
            v_ref[c, 0:HALO, :] = jnp.broadcast_to(v_ref[c, HALO:HALO + 1, :], (HALO, 128))

    links = []

    def attn(t):
        def g_():
            for r0 in range(t * T, (t + 1) * T, RA):
                u = (r0 - t * T) // RA
                q = [q_ref[c, r0:r0 + RA, :] for c in range(4)]
                prev = None
                if t == 0 and u < CHAIN[t]:
                    prev = wo_gate[0]
                elif len(links) >= CHAIN[t]:
                    prev = links[-CHAIN[t]]
                if prev is not None:
                    cvec = pltpu.bitcast(
                        lax.shift_right_logical(pltpu.bitcast(prev, i32), 31) | QBITS, f32)
                    q = [qq * cvec for qq in q]
                else:
                    q = [qq * QSCALE for qq in q]
                logits = []
                for w in range(NW):
                    s = None
                    for c in range(4):
                        kk = k_ref[c, pl.ds(HALO + r0 - DIL * w, RA), :]
                        s = q[c] * kk if s is None else s + q[c] * kk
                    s = s + pltpu.roll(s, 64, 1)
                    s = s + pltpu.roll(s, 32, 1)
                    if w > 0 and r0 < DIL * w:
                        rows = lax.broadcasted_iota(i32, (RA, 128), 0) + r0
                        s = jnp.where(rows >= DIL * w, s, NEG)
                    logits.append(s)
                m = logits[0]
                for w in range(1, NW):
                    m = jnp.maximum(m, logits[w])
                e = [jnp.exp2(l - m) for l in logits]
                den = e[0]
                for w in range(1, NW):
                    den = den + e[w]
                rcp = pltpu.reciprocal(den, approx=True)
                links.append(rcp if t == 0 else e[0])
                for c in range(4):
                    acc = None
                    for w in range(NW):
                        vv = v_ref[c, pl.ds(HALO + r0 - DIL * w, RA), :]
                        acc = e[w] * vv if acc is None else acc + e[w] * vv
                    _st16(o_ref, r0, RA, c * 128, (c + 1) * 128, acc * rcp)
                yield
        return _Gen(g_(), T // RA)

    def wo(t):
        def g_():
            r0 = t * T
            for c in range(4):
                y = jnp.dot(_ld16(o_ref, r0, T), _ld16(wop_ref, 0, D, c * 128, (c + 1) * 128),
                            preferred_element_type=f32)
                h_ref[r0:r0 + T, c * 128:(c + 1) * 128] = (
                    x_ref[r0:r0 + T, c * 128:(c + 1) * 128].astype(f32) + y)
                yield
        return _Gen(g_(), 4)

    def ln2(t):
        def g_():
            for r in range(t * T, (t + 1) * T, RL):
                _st16(hn_ref, r, RL, 0, D, _ln(h_ref[r:r + RL, :]))
                yield
        return _Gen(g_(), T // RL)

    def ffn1(t):
        def g_():
            r0 = t * T
            for f0 in range(0, F, FCH):
                f1 = min(F, f0 + FCH)
                y = lax.dot_general(_ld16(hn_ref, r0, T), _ld16(w1p_ref, f0, f1 - f0),
                                    (((1,), (1,)), ((), ())), preferred_element_type=f32)
                _st16(act_ref, r0, T, f0, f1, _mish(y + bf_ref[:, f0:f1]))
                yield
        return _Gen(g_(), N_F1)

    def ffn2_piece(r0, nr, n0):
        y = jnp.dot(_ld16(act_ref, r0, nr), _ld16(w2p_ref, 0, F, n0, n0 + 128), preferred_element_type=f32)
        out_ref[r0:r0 + nr, n0:n0 + 128] = (h_ref[r0:r0 + nr, n0:n0 + 128] + y).astype(bf16)

    def ffn2(t):
        def g_():
            for n0 in range(0, D, 128):
                for r0 in range(t * T, (t + 1) * T, F2M):
                    ffn2_piece(r0, F2M, n0)
                yield
        return _Gen(g_(), 4)

    xs[0].start()
    wqkv_copy(0).start()
    xs[0].wait()
    xs[1].start()
    _interleave(ln1(0))
    wqkv_copy(0).wait()
    wqkv_copy(1).start()
    q0 = qkv(0, (0,))
    q0.n = 2
    _interleave(permute_part(0), q0)
    xs[1].wait()
    wqkv_copy(2).start()
    q0.n = 4
    _interleave(q0, ln1(1))
    q1 = qkv(1, (0,))
    q1.n = 3
    _interleave(q1)
    wqkv_copy(1).wait()
    xs[2].start()
    wo_copy.start()
    q1.n = 4
    _interleave(permute_part(1), q1)
    _interleave(qkv(0, (1,)))
    k1 = qkv(1, (1,))
    k1.n = 2
    _interleave(k1)
    wqkv_copy(2).wait()
    w1_copy.start()
    b1_copy.start()
    k1.n = 4
    _interleave(permute_part(2), k1)
    _interleave(qkv(0, (2,)))
    halo()
    v1 = qkv(1, (2,))
    v1.n = 1
    _interleave(v1)
    xs[2].wait()
    wo_copy.wait()
    xs[3].start()
    w2_copy.start()
    v1.n = 4
    _interleave(v1, ln1(2), permute_wo())

    for t in range(NT):
        gens = [attn(t)]
        if t == 0:
            gens.append(qkv(2, (0, 1)))
        elif t + 2 < NT:
            gens.append(qkv(t + 2))
        f2 = ffn2(t - 1) if t >= 1 else None
        if t == NT - 1:
            f2.n = 2
            gens.append(f2)
        _interleave(*gens)
        _interleave(wo(t))
        gens = [ln2(t)]
        if t == 0:
            w1_copy.wait()
            b1_copy.wait()
            xs[3].wait()
            xr.start()
            bf_ref[...] = b1_ref[...].astype(f32).reshape(1, F)
            gens += [qkv(2, (2,)), repack(w1t_ref, w1p_ref)]
        else:
            if t == 1:
                _interleave(repack(w2_ref, w2p_ref))
            f2.n = 4
            gens.append(f2)
        if t + 3 < NT:
            gens.append(ln1(t + 3))
        _interleave(*gens)
        if t >= 1:
            out_copy(t - 1).start()
        _interleave(ffn1(t))
        if t == 0:
            w2_copy.wait()
            xr.wait()

    r_last = (NT - 1) * T
    for n0 in range(0, D, 128):
        for r0 in range(r_last, S, TAILM):
            ffn2_piece(r0, TAILM, n0)
            if n0 == D - 128 or r0 + TAILM == S:
                r1, nr = (r0, TAILM) if n0 == D - 128 else (r_last, T)
                pltpu.make_async_copy(out_ref.at[pl.ds(r1, nr), pl.ds(n0, 128)],
                                      out_hbm.at[pl.ds(r1, nr), pl.ds(n0, 128)], sem_o).start()
    pltpu.make_async_copy(out_ref, out_hbm, sem_o).wait()


@jax.jit
def pallas_sequential_preLN__sliding_local_dilated__dense_activation_mish__prompt_kernel(
    A_x: jax.Array,
    A_wqkv: jax.Array,
    A_wo: jax.Array,
    B_x: jax.Array,
    B_w1: jax.Array,
    B_b1: jax.Array,
    B_w2: jax.Array,
):
    del B_x
    hbm = pl.BlockSpec(memory_space=pltpu.HBM)
    out = pl.pallas_call(
        _kernel,
        in_specs=[hbm] * 6,
        out_specs=hbm,
        out_shape=jax.ShapeDtypeStruct((S, D), bf16),
        scratch_shapes=[
            pltpu.VMEM((S, D), bf16),
            pltpu.VMEM((D, 3 * D), bf16),
            pltpu.VMEM((D, D), bf16),
            pltpu.VMEM((F, D), bf16),
            pltpu.VMEM((F,), bf16),
            pltpu.VMEM((F, D), bf16),
            pltpu.VMEM((S, D), bf16),
            pltpu.VMEM((D // 2, 3 * D), i32),
            pltpu.VMEM((D // 2, D), i32),
            pltpu.VMEM((F // 2, D), i32),
            pltpu.VMEM((F // 2, D), i32),
            pltpu.VMEM((1, F), f32),
            pltpu.VMEM((4, D, 128), f32),
            pltpu.VMEM((4, S, 128), f32),
            pltpu.VMEM((4, HALO + S, 128), f32),
            pltpu.VMEM((4, HALO + S, 128), f32),
            pltpu.VMEM((S // 2, D), i32),
            pltpu.VMEM((S // 2, D), i32),
            pltpu.VMEM((S, D), f32),
            pltpu.VMEM((S // 2, D), i32),
            pltpu.VMEM((S // 2, F), i32),
            pltpu.SemaphoreType.DMA((3,)),
        ],
        compiler_params=pltpu.CompilerParams(vmem_limit_bytes=100 * 1024 * 1024),
    )(A_x.reshape(S, D), A_wqkv, A_wo, B_w1.T, B_b1, B_w2)
    return out.reshape(1, S, D)
```

```python
import jax
import jax.numpy as jnp
import numpy as np
from jax import lax
import jax.experimental.pallas as pl
import jax.experimental.pallas.tpu as pltpu

S, D, H, DH, F = 2048, 512, 32, 16, 1376
NW, DIL = 8, 2
HALO = 16
EPS = 1e-5
LOG2E = 1.4426950408889634
QSCALE = (DH ** -0.5) * LOG2E
QBITS = int(np.float32(QSCALE).view(np.int32))
NEG = -1e9 * LOG2E
f32, bf16, i32 = jnp.float32, jnp.bfloat16, jnp.int32

T = 256
NT = S // T
RA = 16
RL = 64
RC = 64
FCH = 128
F2M = 128
TAILM = 64
CHAIN = (4, 5, 5, 5, 5, 5, 5, 5)
N_F1 = len(range(0, F, FCH))


def _ln(x):
    m = jnp.sum(x, axis=-1, keepdims=True) * (1.0 / D)
    d = x - m
    v = jnp.sum(d * d, axis=-1, keepdims=True) * (1.0 / D)
    return d * lax.rsqrt(v + EPS)


def _mish(h):
    n = jnp.exp2(jnp.minimum(h, 20.0) * LOG2E)
    u = n * (n + 2.0)
    return h * u * pltpu.reciprocal(u + 2.0, approx=True)


def _ld16(ref, r0, nr, c0=None, c1=None):
    if c0 is None:
        return pltpu.bitcast(ref[r0 // 2:(r0 + nr) // 2, :], bf16)
    return pltpu.bitcast(ref[r0 // 2:(r0 + nr) // 2, c0:c1], bf16)


def _st16(ref, r0, nr, c0, c1, val):
    ref[r0 // 2:(r0 + nr) // 2, c0:c1] = pltpu.bitcast(val.astype(bf16), i32)


class _Gen:
    def __init__(self, g, n):
        self.g, self.n, self.i = g, n, 0


def _interleave(*gens):
    start = [s.i for s in gens]
    while True:
        live = [k for k, s in enumerate(gens) if s.i < s.n]
        if not live:
            return
        k = min(live, key=lambda k: (gens[k].i - start[k] + 0.5) / (gens[k].n - start[k]))
        next(gens[k].g)
        gens[k].i += 1


def _kernel(x_hbm, wqkv_hbm, wo_hbm, w1t_hbm, b1_hbm, w2_hbm, out_hbm,
            x_ref, wqkv_ref, wo_ref, w1t_ref, b1_ref, w2_ref, out_ref,
            wp_ref, wop_ref, w1p_ref, w2p_ref, bf_ref, tmp_ref, q_ref, k_ref, v_ref,
            xn_ref, o_ref, h_ref, hn_ref, act_ref,
            sems):

    def rows_copy(src, dst, r0, n, sem):
        return pltpu.make_async_copy(src.at[pl.ds(r0, n), :], dst.at[pl.ds(r0, n), :], sem)

    sem_a, sem_b, sem_o = sems.at[0], sems.at[1], sems.at[2]

    def wqkv_copy(p):
        return pltpu.make_async_copy(wqkv_hbm.at[:, pl.ds(p * D, D)],
                                     wqkv_ref.at[:, pl.ds(p * D, D)], (sem_b, sem_b, sem_a)[p])

    wo_copy = pltpu.make_async_copy(wo_hbm, wo_ref, sem_b)
    w1_copy = pltpu.make_async_copy(w1t_hbm, w1t_ref, sem_a)
    b1_copy = pltpu.make_async_copy(b1_hbm, b1_ref, sem_a)
    w2_copy = pltpu.make_async_copy(w2_hbm, w2_ref, sem_b)
    xs = [rows_copy(x_hbm, x_ref, i * T, T, (sem_a, sem_a, sem_b, sem_a)[i]) for i in range(4)]
    xr = rows_copy(x_hbm, x_ref, 4 * T, S - 4 * T, sem_a)

    def out_copy(t):
        return rows_copy(out_ref, out_hbm, t * T, T, sem_o)

    def permute_part(p):
        def g_():
            lane = lax.broadcasted_iota(i32, (RC // 2, 128), 1)
            quad = (lane % 16) // 4
            g = lane // 32
            b = (lane % 32) // 8
            hl = lane % 8
            for c in range(4):
                idx = hl * 16 + 4 * ((b + c) % 4) + g
                for r in range(0, D, RC):
                    blks = [pltpu.bitcast(wqkv_ref[r:r + RC, p * D + bb * 128:p * D + (bb + 1) * 128], i32)
                            for bb in range(4)]
                    xx = blks[(0 - c) % 4]
                    for qd in range(1, 4):
                        xx = jnp.where(quad == qd, blks[(qd - c) % 4], xx)
                    wp_ref[r // 2:(r + RC) // 2, p * D + c * 128:p * D + (c + 1) * 128] = (
                        jnp.take_along_axis(xx, idx, axis=1))
                yield
        return _Gen(g_(), 4)

    wo_gate = []

    def permute_wo():
        def g_():
            for j in range(4):
                for r in range(0, D, 64):
                    tmp_ref[j, r:r + 64, :] = wo_ref[r:r + 64, j * 128:(j + 1) * 128].astype(f32)
                yield
            for j in range(4):
                for c in range(4):
                    for g in range(4):
                        parts = [tmp_ref[j, pl.ds(128 * b + 4 * ((b + c) % 4) + g, 8, stride=16), :]
                                 for b in range(4)]
                        v = jnp.concatenate(parts, axis=0)
                        _st16(wop_ref, c * 128 + 32 * g, 32, j * 128, (j + 1) * 128, v)
                        if j == 3 and c == 3 and g == 3:
                            wo_gate.append(jnp.abs(v[0:RA, :]))
                yield
        return _Gen(g_(), 8)

    def repack(src_ref, dst_ref):
        def g_():
            for r in range(0, F, RC):
                n = min(RC, F - r)
                dst_ref[r // 2:(r + n) // 2, :] = pltpu.bitcast(src_ref[r:r + n, :], i32)
                yield
        return _Gen(g_(), len(range(0, F, RC)))

    def ln1(t):
        def g_():
            for r in range(t * T, (t + 1) * T, RL):
                _st16(xn_ref, r, RL, 0, D, _ln(x_ref[r:r + RL, :].astype(f32)))
                yield
        return _Gen(g_(), T // RL)

    def qkv(t, parts=(0, 1, 2)):
        def g_():
            r0 = t * T
            for p in parts:
                for c in range(4):
                    y = jnp.dot(_ld16(xn_ref, r0, T),
                                _ld16(wp_ref, 0, D, p * D + c * 128, p * D + (c + 1) * 128),
                                preferred_element_type=f32)
                    if p == 0:
                        q_ref[c, r0:r0 + T, :] = y
                    elif p == 1:
                        k_ref[c, HALO + r0:HALO + r0 + T, :] = y
                    else:
                        v_ref[c, HALO + r0:HALO + r0 + T, :] = y
                    yield
        return _Gen(g_(), 4 * len(parts))

    def halo():
        for c in range(4):
            k_ref[c, 0:HALO, :] = jnp.broadcast_to(k_ref[c, HALO:HALO + 1, :], (HALO, 128))
            v_ref[c, 0:HALO, :] = jnp.broadcast_to(v_ref[c, HALO:HALO + 1, :], (HALO, 128))

    links = []

    def attn(t):
        def g_():
            for r0 in range(t * T, (t + 1) * T, RA):
                u = (r0 - t * T) // RA
                q = [q_ref[c, r0:r0 + RA, :] for c in range(4)]
                prev = None
                if t == 0 and u < CHAIN[t]:
                    prev = wo_gate[0]
                elif len(links) >= CHAIN[t]:
                    prev = links[-CHAIN[t]]
                if prev is not None:
                    cvec = pltpu.bitcast(
                        lax.shift_right_logical(pltpu.bitcast(prev, i32), 31) | QBITS, f32)
                    q = [qq * cvec for qq in q]
                else:
                    q = [qq * QSCALE for qq in q]
                logits = []
                for w in range(NW):
                    s = None
                    for c in range(4):
                        kk = k_ref[c, pl.ds(HALO + r0 - DIL * w, RA), :]
                        s = q[c] * kk if s is None else s + q[c] * kk
                    s = s + pltpu.roll(s, 64, 1)
                    s = s + pltpu.roll(s, 32, 1)
                    if w > 0 and r0 < DIL * w:
                        rows = lax.broadcasted_iota(i32, (RA, 128), 0) + r0
                        s = jnp.where(rows >= DIL * w, s, NEG)
                    logits.append(s)
                m = logits[0]
                for w in range(1, NW):
                    m = jnp.maximum(m, logits[w])
                e = [jnp.exp2(l - m) for l in logits]
                den = e[0]
                for w in range(1, NW):
                    den = den + e[w]
                rcp = pltpu.reciprocal(den, approx=True)
                links.append(rcp if t == 0 else e[0])
                for c in range(4):
                    acc = None
                    for w in range(NW):
                        vv = v_ref[c, pl.ds(HALO + r0 - DIL * w, RA), :]
                        acc = e[w] * vv if acc is None else acc + e[w] * vv
                    _st16(o_ref, r0, RA, c * 128, (c + 1) * 128, acc * rcp)
                yield
        return _Gen(g_(), T // RA)

    def wo(t):
        def g_():
            r0 = t * T
            for c in range(4):
                y = jnp.dot(_ld16(o_ref, r0, T), _ld16(wop_ref, 0, D, c * 128, (c + 1) * 128),
                            preferred_element_type=f32)
                h_ref[r0:r0 + T, c * 128:(c + 1) * 128] = (
                    x_ref[r0:r0 + T, c * 128:(c + 1) * 128].astype(f32) + y)
                yield
        return _Gen(g_(), 4)

    def ln2(t):
        def g_():
            for r in range(t * T, (t + 1) * T, RL):
                _st16(hn_ref, r, RL, 0, D, _ln(h_ref[r:r + RL, :]))
                yield
        return _Gen(g_(), T // RL)

    def ffn1(t):
        def g_():
            r0 = t * T
            for f0 in range(0, F, FCH):
                f1 = min(F, f0 + FCH)
                y = lax.dot_general(_ld16(hn_ref, r0, T), _ld16(w1p_ref, f0, f1 - f0),
                                    (((1,), (1,)), ((), ())), preferred_element_type=f32)
                _st16(act_ref, r0, T, f0, f1, _mish(y + bf_ref[:, f0:f1]))
                yield
        return _Gen(g_(), N_F1)

    def ffn2_piece(r0, nr, n0):
        y = jnp.dot(_ld16(act_ref, r0, nr), _ld16(w2p_ref, 0, F, n0, n0 + 128), preferred_element_type=f32)
        out_ref[r0:r0 + nr, n0:n0 + 128] = (h_ref[r0:r0 + nr, n0:n0 + 128] + y).astype(bf16)

    def ffn2(t):
        def g_():
            for n0 in range(0, D, 128):
                for r0 in range(t * T, (t + 1) * T, F2M):
                    ffn2_piece(r0, F2M, n0)
                yield
        return _Gen(g_(), 4)

    xs[0].start()
    wqkv_copy(0).start()
    xs[0].wait()
    xs[1].start()
    _interleave(ln1(0))
    wqkv_copy(0).wait()
    wqkv_copy(1).start()
    q0 = qkv(0, (0,))
    q0.n = 2
    _interleave(permute_part(0), q0)
    xs[1].wait()
    wqkv_copy(2).start()
    q0.n = 4
    _interleave(q0, ln1(1))
    q1 = qkv(1, (0,))
    q1.n = 3
    _interleave(q1)
    wqkv_copy(1).wait()
    xs[2].start()
    wo_copy.start()
    q1.n = 4
    _interleave(permute_part(1), q1)
    _interleave(qkv(0, (1,)))
    k1 = qkv(1, (1,))
    k1.n = 2
    _interleave(k1)
    wqkv_copy(2).wait()
    w1_copy.start()
    b1_copy.start()
    k1.n = 4
    _interleave(permute_part(2), k1)
    _interleave(qkv(0, (2,)))
    halo()
    xs[2].wait()
    wo_copy.wait()
    xs[3].start()
    w2_copy.start()
    _interleave(qkv(1, (2,)), ln1(2), permute_wo())

    for t in range(NT):
        gens = [attn(t)]
        if t == 0:
            gens.append(qkv(2, (0, 1)))
        elif t + 2 < NT:
            gens.append(qkv(t + 2))
        f2 = ffn2(t - 1) if t >= 1 else None
        if t == NT - 1:
            f2.n = 2
            gens.append(f2)
        _interleave(*gens)
        _interleave(wo(t))
        gens = [ln2(t)]
        if t == 0:
            w1_copy.wait()
            b1_copy.wait()
            xs[3].wait()
            xr.start()
            bf_ref[...] = b1_ref[...].astype(f32).reshape(1, F)
            gens += [qkv(2, (2,)), repack(w1t_ref, w1p_ref)]
        else:
            if t == 1:
                _interleave(repack(w2_ref, w2p_ref))
            f2.n = 4
            gens.append(f2)
        if t + 3 < NT:
            gens.append(ln1(t + 3))
        _interleave(*gens)
        if t >= 1:
            out_copy(t - 1).start()
        _interleave(ffn1(t))
        if t == 0:
            w2_copy.wait()
            xr.wait()

    r_last = (NT - 1) * T
    for n0 in range(0, D, 128):
        for r0 in range(r_last, S, TAILM):
            ffn2_piece(r0, TAILM, n0)
            if n0 == D - 128 or r0 + TAILM == S:
                r1, nr = (r0, TAILM) if n0 == D - 128 else (r_last, T)
                pltpu.make_async_copy(out_ref.at[pl.ds(r1, nr), pl.ds(n0, 128)],
                                      out_hbm.at[pl.ds(r1, nr), pl.ds(n0, 128)], sem_o).start()
    pltpu.make_async_copy(out_ref, out_hbm, sem_o).wait()


@jax.jit
def pallas_sequential_preLN__sliding_local_dilated__dense_activation_mish__prompt_kernel(
    A_x: jax.Array,
    A_wqkv: jax.Array,
    A_wo: jax.Array,
    B_x: jax.Array,
    B_w1: jax.Array,
    B_b1: jax.Array,
    B_w2: jax.Array,
):
    del B_x
    hbm = pl.BlockSpec(memory_space=pltpu.HBM)
    out = pl.pallas_call(
        _kernel,
        in_specs=[hbm] * 6,
        out_specs=hbm,
        out_shape=jax.ShapeDtypeStruct((S, D), bf16),
        scratch_shapes=[
            pltpu.VMEM((S, D), bf16),
            pltpu.VMEM((D, 3 * D), bf16),
            pltpu.VMEM((D, D), bf16),
            pltpu.VMEM((F, D), bf16),
            pltpu.VMEM((F,), bf16),
            pltpu.VMEM((F, D), bf16),
            pltpu.VMEM((S, D), bf16),
            pltpu.VMEM((D // 2, 3 * D), i32),
            pltpu.VMEM((D // 2, D), i32),
            pltpu.VMEM((F // 2, D), i32),
            pltpu.VMEM((F // 2, D), i32),
            pltpu.VMEM((1, F), f32),
            pltpu.VMEM((4, D, 128), f32),
            pltpu.VMEM((4, S, 128), f32),
            pltpu.VMEM((4, HALO + S, 128), f32),
            pltpu.VMEM((4, HALO + S, 128), f32),
            pltpu.VMEM((S // 2, D), i32),
            pltpu.VMEM((S // 2, D), i32),
            pltpu.VMEM((S, D), f32),
            pltpu.VMEM((S // 2, D), i32),
            pltpu.VMEM((S // 2, F), i32),
            pltpu.SemaphoreType.DMA((3,)),
        ],
        compiler_params=pltpu.CompilerParams(vmem_limit_bytes=100 * 1024 * 1024),
    )(A_x.reshape(S, D), A_wqkv, A_wo, B_w1.T, B_b1, B_w2)
    return out.reshape(1, S, D)
```
